```python
import os as _os
_os.environ.setdefault("JAX_PLATFORMS", "cpu")
import jax
import jax.numpy as jnp

def _softmax(x, axis=-1):
    return jax.nn.softmax(x, axis=axis)
def _gelu(x):
    return jax.nn.gelu(x, approximate=True)
def _silu(x):
    return jax.nn.silu(x)
def _sigmoid(x):
    return jax.nn.sigmoid(x)
def _layernorm(x, axis=-1, eps=1e-5):
    m = jnp.mean(x, axis=axis, keepdims=True)
    v = jnp.var(x, axis=axis, keepdims=True)
    return (x - m) / jnp.sqrt(v + eps)
def _scatter_add(tgt, idx, src, axis=0):
    return tgt.at[idx].add(src)
def _segment_sum(src, seg, n):
    return jax.ops.segment_sum(src, seg, n)
class _Rng:
    def __init__(self, key):
        self._k = key
    def _next(self):
        self._k, sub = jax.random.split(self._k)
        return sub
    def normal(self, shape):
        return jax.random.normal(self._next(), shape, dtype=jnp.bfloat16)
    def randint(self, lo, hi, shape):
        return jax.random.randint(self._next(), shape, lo, hi, dtype=jnp.int32)
    def uniform(self, shape, lo=0.0, hi=1.0):
        return jax.random.uniform(self._next(), shape, jnp.bfloat16, lo, hi)
    def permutation(self, n):
        return jax.random.permutation(self._next(), n)


kernel_name = 'concat_heads__gqa_block_cached__mha_block_cached__near_ridge'

def setup_inputs():
    _rng = _Rng(jax.random.key(int.from_bytes(__import__("os").urandom(4), "little")))
    _w = (lambda a: (lambda t: t.astype(jnp.bfloat16) if jnp.issubdtype(t.dtype, jnp.floating) else t)(jnp.asarray(a)))
    def _A_setup():
        B, Sq, D = 8, 112, 448
        Hq, Hkv, Sk, Dh = 16, 8, 512, 256
        assert Hq % Hkv == 0, (Hq, Hkv)
        return {
            "x": _w((lambda *s: _rng.normal(s) * 0.8)(B, Sq, D)),
            "k_cache": _w((lambda *s: _rng.normal(s) * 0.8)(B, Hkv, Sk, Dh)),
            "v_cache": _w((lambda *s: _rng.normal(s) * 0.05)(B, Hkv, Sk, Dh)),
            "wq": _w((lambda *s: _rng.normal(s) * 0.8)(D, Hq * Dh) * (D ** -0.5)),
            "wo": _w((lambda *s: _rng.normal(s) * 0.05)(Hq * Dh, D) * ((Hq * Dh) ** -0.5)),
        }
    _A_in = _A_setup()

    def _B_setup():
        B, Sq, D = 8, 112, 448
        H, Sk, Dh = 16, 512, 256
        return {
            "x": _w((lambda *s: _rng.normal(s) * 0.8)(B, Sq, D)),
            "k_cache": _w((lambda *s: _rng.normal(s) * 0.8)(B, H, Sk, Dh)),
            "v_cache": _w((lambda *s: _rng.normal(s) * 0.05)(B, H, Sk, Dh)),
            "wq": _w((lambda *s: _rng.normal(s) * 0.8)(D, H * Dh) * (D ** -0.5)),
            "wo": _w((lambda *s: _rng.normal(s) * 0.05)(H * Dh, D) * ((H * Dh) ** -0.5)),
        }
    _B_in = _B_setup()

    return {
        "A_x": _A_in["x"],
        "A_k_cache": _A_in["k_cache"],
        "A_v_cache": _A_in["v_cache"],
        "A_wq": _A_in["wq"],
        "A_wo": _A_in["wo"],
        "B_x": _B_in["x"],
        "B_k_cache": _B_in["k_cache"],
        "B_v_cache": _B_in["v_cache"],
        "B_wq": _B_in["wq"],
        "B_wo": _B_in["wo"],
    }

def reference(A_x, A_k_cache, A_v_cache, A_wq, A_wo, B_x, B_k_cache, B_v_cache, B_wq, B_wo):
    def _A_ref(x, k_cache, v_cache, wq, wo):
        B, Sq, D = x.shape
        Hq, Dh = 16, 256
        Hkv = k_cache.shape[1]
        rep = Hq // Hkv
        q = (lambda x, *d: x.transpose(*d))((x @ wq).reshape(B, Sq, Hq, Dh), 0, 2, 1, 3)
        k = jnp.repeat(k_cache, rep, axis=1)
        v = jnp.repeat(v_cache, rep, axis=1)
        scores = jnp.einsum("bhqd,bhkd->bhqk", q, k) * (Dh ** -0.5)
        p = _softmax(scores, axis=-1)
        o = jnp.einsum("bhqk,bhkd->bhqd", p, v)
        return (lambda x, *d: x.transpose(*d))(o, 0, 2, 1, 3).reshape(B, Sq, Hq * Dh) @ wo

    def _B_ref(x, k_cache, v_cache, wq, wo):
        B, Sq, D = x.shape
        H, Dh = 16, 256
        q = (lambda x, *d: x.transpose(*d))((x @ wq).reshape(B, Sq, H, Dh), 0, 2, 1, 3)
        scores = jnp.einsum("bhqd,bhkd->bhqk", q, k_cache) * (Dh ** -0.5)
        p = _softmax(scores, axis=-1)
        o = jnp.einsum("bhqk,bhkd->bhqd", p, v_cache)
        return (lambda x, *d: x.transpose(*d))(o, 0, 2, 1, 3).reshape(B, Sq, H * Dh) @ wo

    a = _A_ref(A_x, A_k_cache, A_v_cache, A_wq, A_wo)
    b = _B_ref(B_x, B_k_cache, B_v_cache, B_wq, B_wo)
    return jnp.concatenate([a, b], axis=-1)
```

```python
import math
import jax
import jax.numpy as jnp
from jax import lax
import jax.experimental.pallas as pl
import jax.experimental.pallas.tpu as pltpu

NB, SQ, D, SK, DH = 8, 112, 448, 512, 256
M = NB * SQ
NT = (((1,), (1,)), ((), ()))
F32, BF = jnp.float32, jnp.bfloat16
QSCALE = DH ** -0.5 * math.log2(math.e)
NSTEP, NPAIR, APAIR = 16, 96, 32

ORD = {
 0: "S0 a1 w0 k0 Q1 S1 a2 c0 v0 X0 P0 Q2 S2 a3 c1 f0 k1 v1 X1 P1 Q3 S3 a4 c2 k2 X2 P2 O0 Q4 S4 a5 c3 v2 u0 X3 P3 T0 O1 Q5 S5 a6 c4 k3 v3 X4 P4 T1 O2 Q6 S6 a7 c5 k4 X5 P5 T2 O3 Q7 S7 a8 c6 c7 e0 v4 k5 v5 X6 P6 T3 O4 X7 P7 T4 O5 Q8 T5 O6 T6",
 1: "S0 Q1 S1 a2 a3 c0 c1 f0 w0 k0 v0 k1 X0 P0 Q2 S2 X1 P1 Q3 S3 a4 a5 c2 c3 v1 k2 v2 u0 X2 P2 O0 Q4 S4 X3 P3 T0 O1 Q5 S5 a6 a7 c4 c5 k3 v3 k4 X4 P4 T1 O2 Q6 S6 X5 P5 T2 O3 Q7 S7 a8 a9 c6 c7 e0 v4 k5 v5 X6 P6 T3 O4 X7 P7 T4 O5 Q8 T5 O6 T6",
 2: "a0 a1 a2 a3 a4 c0 c1 c2 c3 f0 w0 k0 v0 k1 v1 k2 v2 S0 Q1 S1 X0 P0 Q2 S2 X1 P1 Q3 S3 X2 P2 O0 Q4 S4 a5 a6 a7 c4 c5 c6 c7 e0 u0 k3 v3 k4 v4 k5 v5 X3 P3 T0 O1 Q5 S5 X4 P4 T1 O2 Q6 S6 X5 P5 T2 O3 Q7 S7 X6 P6 T3 O4 X7 P7 T4 O5 Q8 T5 O6 T6",
}

def check(ops, lead, R):
    iss = {'k': set(range(lead)), 'v': set(range(lead)), 'w': {0}, 'u': {0}}
    done = {'k': set(), 'v': set(), 'w': {0}, 'u': set()}
    used = {'k': {}, 'v': {}}
    pair = lambda j, b: 4 * j + b // 2 if j < 8 else 8 * j - APAIR + b
    def wait(st, n):
        assert n in iss[st] and n not in done[st], ('bad wait', st, n); done[st].add(n)
    for op in ops:
        if op[0] in 'ac' and int(op[1:]) >= NB and (int(op[1:]) - NB) % 2 == 0:
            wait('k' if op[0] == 'a' else 'v', (int(op[1:]) - NB) // 2)
    for j in range(NSTEP):
        for op in ops:
            c, i = op[0], int(op[1:])
            if c in 'kv':
                n = 6 * j + i + lead
                if n < NPAIR:
                    assert n - R < 0 or used[c].get(n - R, 0) == (2 if n - R < APAIR else 1), ('ring', c, n); iss[c].add(n)
            elif c in 'wu':
                if j + 1 < NSTEP: iss[c].add(j + 1)
            elif c in 'ac':
                jj, b = (j + 1, i - NB) if i >= NB else (j, i)
                if jj < NSTEP and (b % 2 == 0 or jj >= 8): wait('k' if c == 'a' else 'v', pair(jj, b))
            elif c == 'e':
                if j + 1 < NSTEP: wait('w', j + 1)
            elif c == 'f': wait('u', j)
            elif c in 'SP':
                st = 'k' if c == 'S' else 'v'; assert pair(j, i) in done[st], ('use', op, j); used[st][pair(j, i)] = used[st].get(pair(j, i), 0) + 1
            elif c == 'O': assert j in done['u']
            elif c == 'Q' and i >= NB: assert min(j + 1, NSTEP - 1) in done['w']
    for st in iss: assert iss[st] == done[st] and len(iss[st]) == (NPAIR if st in 'kv' else NSTEP), st

def make(order=0, lead=2, R=32, stage='bf', dma=True, flags=None, exp=''):
    ops = (ORD[order] if isinstance(order, int) else order).split()
    LA = max(int(o[1:]) for o in ops if o[0] == 'Q') - 7
    if dma: check(ops, lead, R)
    if exp == 'dmaonly': ops = [o for o in ops if o[0] not in 'SXPQOT']
    if stage == 'none': ops = [o for o in ops if o[0] != 'T']

    def kern(xa_h, ka_h, va_h, wqa_h, woa_h, xb_h, kb_h, vb_h, wqb_h, wob_h, out_h,
             x, wq, wo, kr, vr, q, o, acc, stg, s_x, s_wq, s_wo, s_k, s_v, s_o):
        def pair_start(n, a_h, b_h, ring, sem):
            slot = n & (R - 1)
            def from_a():
                pltpu.make_async_copy(a_h.at[pl.ds(2 * (n & 3), 2), n >> 2], ring.at[slot], sem.at[slot]).start()
            if isinstance(n, int):
                assert n < APAIR
                return from_a()
            pl.when(n < APAIR)(from_a)
            @pl.when(jnp.logical_and(n >= APAIR, n < NPAIR))
            def _():
                m = n - APAIR
                pltpu.make_async_copy(b_h.at[m & 7, pl.ds(2 * (m >> 3), 2)], ring.at[slot], sem.at[slot]).start()
        def ring_wait(ring, sem, slot):
            pltpu.make_async_copy(ring.at[slot], ring.at[slot], sem.at[slot]).wait()
        def w_start(j, a_h, b_h, buf, sem):
            if isinstance(j, int):
                return pltpu.make_async_copy(a_h.at[:, pl.ds(j * 512, 512)], buf.at[j], sem.at[j]).start()
            c = pl.ds(pl.multiple_of((j & 7) * 512, 512), 512)
            @pl.when(j < 8)
            def _(): pltpu.make_async_copy(a_h.at[:, c], buf.at[j], sem.at[j]).start()
            @pl.when(jnp.logical_and(j >= 8, j < NSTEP))
            def _(): pltpu.make_async_copy(b_h.at[:, c], buf.at[j], sem.at[j]).start()
        def qproj(br, j, b):
            r = jnp.dot(x[br, pl.ds(b * SQ, SQ)], wq[j], preferred_element_type=F32)
            q[b] = (r * QSCALE).astype(BF)
        def out_copy(t):
            r = pl.ds(t * 128, 128)
            return pltpu.make_async_copy(stg.at[r], out_h.at[r], s_o.at[t])

        X0 = LA * SQ
        cx0 = pltpu.make_async_copy(xa_h.at[pl.ds(0, X0)], x.at[0, pl.ds(0, X0)], s_x.at[0])
        cx1 = pltpu.make_async_copy(xa_h.at[pl.ds(X0, M - X0)], x.at[0, pl.ds(X0, M - X0)], s_x.at[1])
        cx2 = pltpu.make_async_copy(xb_h, x.at[1], s_x.at[2])
        cx0.start(); w_start(0, wqa_h, wqb_h, wq, s_wq)
        pair_start(0, ka_h, kb_h, kr, s_k)
        acc[...] = jnp.zeros_like(acc)
        cx0.wait(); ring_wait(wq, s_wq, 0)
        cx1.start(); pair_start(0, va_h, vb_h, vr, s_v)
        for b in range(LA): qproj(0, 0, b)
        for n in range(1, lead):
            pair_start(n, ka_h, kb_h, kr, s_k); pair_start(n, va_h, vb_h, vr, s_v)
        w_start(0, woa_h, wob_h, wo, s_wo)
        cx1.wait()
        if dma:
            for op in ops:
                if op[0] in 'ac' and int(op[1:]) >= NB and (int(op[1:]) - NB) % 2 == 0:
                    n = (int(op[1:]) - NB) // 2
                    ring_wait(*((kr, s_k) if op[0] == 'a' else (vr, s_v)), n)
        if not dma:
            cx2.start(); cx2.wait(); ring_wait(wo, s_wo, 0)
            for n in range(lead): ring_wait(kr, s_k, n); ring_wait(vr, s_v, n)

        def step(j, _):
            br = j >> 3
            jn = jnp.minimum(j + 1, NSTEP - 1)
            s, p, linv = {}, {}, {}
            def slot_of(b):
                return jnp.where(br == 0, 4 * j + b // 2, 8 * j - APAIR + b) & (R - 1)
            def kv_wait(ring, sem, b):
                if not dma: return
                if b >= NB:
                    jj, bb = j + 1, b - NB
                    sl = jnp.where(jj < 8, 4 * jj + bb // 2, 8 * jj - APAIR + bb) & (R - 1)
                    cond = jj < NSTEP if bb % 2 == 0 else jnp.logical_and(jj >= 8, jj < NSTEP)
                    pl.when(cond)(lambda: ring_wait(ring, sem, sl))
                elif b % 2 == 0: ring_wait(ring, sem, slot_of(b))
                else: pl.when(br == 1)(lambda: ring_wait(ring, sem, slot_of(b)))
            def S(b):
                s[b] = [lax.dot_general(q[b, :, pl.ds(h * DH, DH)], kr[slot_of(b), jnp.where(br == 0, b % 2, h)], NT,
                                        preferred_element_type=F32) for h in range(2)]
            def X(b):
                p[b], linv[b] = [], []
                for sv in s[b]:
                    e = jnp.exp2(sv - jnp.max(sv, axis=-1, keepdims=True))
                    p[b].append(e.astype(BF)); linv[b].append(1.0 / jnp.sum(e, axis=-1, keepdims=True))
            def P(b):
                for h in range(2):
                    ov = jnp.dot(p[b][h], vr[slot_of(b), jnp.where(br == 0, b % 2, h)], preferred_element_type=F32)
                    o[pl.ds(b * SQ, SQ), pl.ds(h * DH, DH)] = (ov * linv[b][h]).astype(BF)
            def Q(b):
                if b < NB: return qproj(br, j, b)
                qproj(jn >> 3, jn, b - NB)
            def O(t):
                c = pl.ds(t * 128, 128)
                r = pl.ds(pl.multiple_of(br * D, 64), D)
                acc[r, c] += lax.dot_general(wo[j], o[c], NT, preferred_element_type=F32)
            def T(t):
                c = pl.ds(t * 128, 128)
                r = pl.ds(pl.multiple_of(br * 384, 128), 512)
                a = acc[r, c]
                stg[c, r] = a.astype(BF).T if stage == 'bf' else a.T.astype(BF)
                pl.when(j == NSTEP - 1)(lambda: out_copy(t).start())
            def ustart(n, b_h, ring, sem):
                pltpu.make_async_copy(b_h.at[n % 8, pl.ds(2 * ((n // 8) % 8), 2)], ring.at[n & (R - 1)], sem.at[n & (R - 1)]).start()
            def k_(i):
                if dma: pair_start(6 * j + i + lead, ka_h, kb_h, kr, s_k)
            def v_(i):
                if dma: pair_start(6 * j + i + lead, va_h, vb_h, vr, s_v)
            def w_(i):
                if dma:
                    w_start(j + 1, wqa_h, wqb_h, wq, s_wq)
                    pl.when(j == 2)(cx2.start)
            def u_(i):
                if dma: w_start(j + 1, woa_h, wob_h, wo, s_wo)
            def e_(i):
                if dma:
                    pl.when(j < NSTEP - 1)(lambda: ring_wait(wq, s_wq, jn))
                    pl.when(j == 7)(cx2.wait)
            def f_(i):
                if dma: ring_wait(wo, s_wo, j)
            fn = dict(a=lambda b: kv_wait(kr, s_k, b), c=lambda b: kv_wait(vr, s_v, b), e=e_, f=f_, S=S, X=X, P=P, Q=Q, O=O, T=T, k=k_, v=v_, w=w_, u=u_)
            for op in ops: fn[op[0]](int(op[1:]))
        lax.fori_loop(0, NSTEP, step, None)
        if stage == 'none':
            for t in range(7):
                c = pl.ds(t * 128, 128)
                stg[c] = acc[:, c].astype(BF).T
                out_copy(t).start()
        for t in range(7): out_copy(t).wait()

    def f(A_x, A_k_cache, A_v_cache, A_wq, A_wo, B_x, B_k_cache, B_v_cache, B_wq, B_wo):
        dsem = pltpu.SemaphoreType.DMA
        out = pl.pallas_call(
            kern, out_shape=jax.ShapeDtypeStruct((M, 2 * D), BF),
            in_specs=[pl.BlockSpec(memory_space=pl.ANY)] * 10, out_specs=pl.BlockSpec(memory_space=pl.ANY),
            scratch_shapes=[
                pltpu.VMEM((2, M, D), BF), pltpu.VMEM((NSTEP, D, 512), BF), pltpu.VMEM((NSTEP, D, 512), BF),
                pltpu.VMEM((R, 2, SK, DH), BF), pltpu.VMEM((R, 2, SK, DH), BF),
                pltpu.VMEM((NB, SQ, 2 * DH), BF), pltpu.VMEM((M, 2 * DH), BF),
                pltpu.VMEM((2 * D, M), F32), pltpu.VMEM((M, 2 * D), BF),
                dsem((3,)), dsem((NSTEP,)), dsem((NSTEP,)), dsem((R,)), dsem((R,)), dsem((7,)),
            ],
            compiler_params=pltpu.CompilerParams(vmem_limit_bytes=100 * 2**20, flags=flags, disable_bounds_checks=True),
        )(A_x.reshape(M, D), A_k_cache, A_v_cache, A_wq, A_wo.T, B_x.reshape(M, D), B_k_cache, B_v_cache, B_wq, B_wo.T)
        return out.reshape(NB, SQ, 2 * D)
    return f


_impl = make(order=0, stage='none', lead=3, flags={'XLA_TPU_RESCHEDULE_DMA_DONES': True})


@jax.jit
def pallas_concat_heads__gqa_block_cached__mha_block_cached__near_ridge_kernel(
    A_x, A_k_cache, A_v_cache, A_wq, A_wo, B_x, B_k_cache, B_v_cache, B_wq, B_wo):
    return _impl(A_x, A_k_cache, A_v_cache, A_wq, A_wo, B_x, B_k_cache, B_v_cache, B_wq, B_wo)
```

```python
import math

import jax
import jax.numpy as jnp
from jax import lax
import jax.experimental.pallas as pl
import jax.experimental.pallas.tpu as pltpu

_NB, _SQ, _D, _SK, _DH = 8, 112, 448, 512, 256
_M = _NB * _SQ
_W = 2 * _DH
_NSTEP = 16
_A_PAIRS, _NPAIR = 32, 96
_PAIRS_PER_STEP = _NPAIR // _NSTEP
_RING = 32
_X_CUTS = (0, 2, 4, 8)
_XB_START, _XB_WAIT = 4, 7
_LO = 384
_HI = 2 * _D - _LO
_NTILE = _M // 128

_S_K, _S_V = 0, _RING
_S_WQ, _S_WO = 2 * _RING, 2 * _RING + _NSTEP
_S_X = 2 * _RING + 2 * _NSTEP
_S_HI = _S_X + 4
_S_LO = _S_HI + _NTILE
_NSEM = _S_LO + 2

_Q_SCALE = _DH**-0.5 * math.log2(math.e)
_NT = (((1,), (1,)), ((), ()))

_PROLOGUE = "w0 x0 k0 Z0 y0 v0 x1 e0 k1 Q0 a0 v1"
_STEP = """
    S0 a1 u0 k2                 Q1
    S1 a2 c0 x2 v2 y1           X0 P0 Q2
    S2 a3 c1 k3 v3              X1 P1 Q3
    S3 a4 c2 f0 y2 w1 k4        X2 P2 O0 Q4
    S4 a5 c3 v4 k5              X3 P3 O1 Q5
    S5 a6 c4 v5                 X4 P4 O2 Q6
    S6 a7 c5 k6 v6              X5 P5 O3 Q7
    S7 a8 c6 c7 e1 k7 v7        X6 P6 O4 X7 P7 O5 Q8 O6
"""
_LAST_STEP = """
    S0 a1 u0 k2                 Q1 L0
    S1 a2 c0 k3                 X0 P0 Q2 L1
    S2 a3 c1 v2                 X1 P1 Q3 L2 L3
    S3 a4 c2 f0 k4 v3           X2 P2 O0 H0 Q4 L4
    S4 a5 c3 k5                 X3 P3 O1 H1 Q5 L5
    S5 a6 c4 v4                 X4 P4 O2 H2 Q6 L6
    S6 v5 c5                    X5 P5 O3 H3 Q7 h0 a7
    S7 h1 c6 h2                 X6 P6 O4 h3 l0 X7 O5 H4 h4 l1 c7 P7 H5 h5 O6 H6 h6
"""


def _when(cond, fn):
    if isinstance(cond, bool):
        if cond:
            fn()
    else:
        pl.when(cond)(fn)


def _select(cond, a, b):
    if isinstance(cond, bool):
        return a if cond else b
    return jnp.where(cond, a, b)


def _aligned(i, n):
    return i if isinstance(i, int) else pl.multiple_of(i, n)


def _kernel(
    xa_hbm, ka_hbm, va_hbm, wqa_hbm, woa_hbm,
    xb_hbm, kb_hbm, vb_hbm, wqb_hbm, wob_hbm,
    out_hbm,
    x_buf, wq_buf, wo_buf, k_ring, v_ring, q_buf, o_buf, acc, lo_buf, hi_buf, sems,
):
    f32, bf16 = jnp.float32, jnp.bfloat16

    def start_pair(n, a_hbm, b_hbm, ring, sem0):
        slot, m = n & (_RING - 1), n - _A_PAIRS

        def from_a():
            src = a_hbm.at[pl.ds(2 * (n & 3), 2), n >> 2]
            pltpu.make_async_copy(src, ring.at[slot], sems.at[sem0 + slot]).start()

        def from_b():
            src = b_hbm.at[m & 7, pl.ds(2 * (m >> 3), 2)]
            pltpu.make_async_copy(src, ring.at[slot], sems.at[sem0 + slot]).start()

        _when(n < _A_PAIRS, from_a)
        _when((n >= _A_PAIRS) & (n < _NPAIR), from_b)

    def start_weights(j, a_hbm, b_hbm, buf, sem0):
        cols = pl.ds(_aligned((j & 7) * _W, _W), _W)

        def start(src):
            pltpu.make_async_copy(src.at[:, cols], buf.at[j], sems.at[sem0 + j]).start()

        _when(j < 8, lambda: start(a_hbm))
        _when(j >= 8, lambda: start(b_hbm))

    def wait_slot(buf, sem0, slot):
        pltpu.make_async_copy(buf.at[slot], buf.at[slot], sems.at[sem0 + slot]).wait()

    def xa_copy(i):
        rows = pl.ds(_X_CUTS[i] * _SQ, (_X_CUTS[i + 1] - _X_CUTS[i]) * _SQ)
        return pltpu.make_async_copy(xa_hbm.at[rows], x_buf.at[0, rows], sems.at[_S_X + i])

    def xb_copy():
        return pltpu.make_async_copy(xb_hbm, x_buf.at[1], sems.at[_S_X + 3])

    def lo_copy(i):
        rows = pl.ds(i * (_M // 2), _M // 2)
        dst = out_hbm.at[rows, pl.ds(0, _LO)]
        return pltpu.make_async_copy(lo_buf.at[rows], dst, sems.at[_S_LO + i])

    def hi_copy(t):
        rows = pl.ds(t * 128, 128)
        dst = out_hbm.at[rows, pl.ds(_LO, _HI)]
        return pltpu.make_async_copy(hi_buf.at[rows], dst, sems.at[_S_HI + t])

    def run(j, program):
        last = isinstance(j, int) and j == _NSTEP - 1
        scores, probs, inv_sum, proj = {}, {}, {}, {}

        def wrap(b):
            return (j + 1, b - _NB) if b >= _NB else (j, b)

        def slot_of(jj, b):
            return _select(jj < 8, 4 * jj + b // 2, 8 * jj - _A_PAIRS + b) & (_RING - 1)

        def kv_block(ring, b, h):
            return ring[slot_of(j, b), _select(j < 8, b % 2, h)]

        def wait_kv(ring, sem0, b):
            jj, b = wrap(b)
            _when(True if b % 2 == 0 else jj >= 8, lambda: wait_slot(ring, sem0, slot_of(jj, b)))

        def q_proj(b):
            jj, b = wrap(b)
            x = x_buf[jj >> 3, pl.ds(b * _SQ, _SQ)]
            q = jnp.dot(x, wq_buf[jj], preferred_element_type=f32)
            q_buf[b] = (q * _Q_SCALE).astype(bf16)

        def qk(b):
            scores[b] = [
                lax.dot_general(
                    q_buf[b, :, pl.ds(h * _DH, _DH)], kv_block(k_ring, b, h), _NT,
                    preferred_element_type=f32,
                )
                for h in range(2)
            ]

        def softmax(b):
            probs[b], inv_sum[b] = [], []
            for s in scores[b]:
                e = jnp.exp2(s - jnp.max(s, axis=-1, keepdims=True))
                probs[b].append(e.astype(bf16))
                inv_sum[b].append(1.0 / jnp.sum(e, axis=-1, keepdims=True))

        def pv(b):
            for h in range(2):
                o = jnp.dot(probs[b][h], kv_block(v_ring, b, h), preferred_element_type=f32)
                o_buf[pl.ds(b * _SQ, _SQ), pl.ds(h * _DH, _DH)] = (o * inv_sum[b][h]).astype(bf16)

        def o_proj(t):
            tok = pl.ds(t * 128, 128)
            d = lax.dot_general(wo_buf[j], o_buf[tok], _NT, preferred_element_type=f32)
            if last:
                proj[t] = d
            else:
                acc[pl.ds(_aligned((j >> 3) * _D, 64), _D), tok] += d

        def stage_lo(t):
            tok = pl.ds(t * 128, 128)
            lo_buf[tok] = acc[pl.ds(0, _LO), tok].astype(bf16).T

        def stage_hi(t):
            tok = pl.ds(t * 128, 128)
            parts = [acc[pl.ds(_LO, _D - _LO), tok], acc[pl.ds(_D, _D), tok] + proj[t]]
            hi_buf[tok] = jnp.concatenate(parts, axis=0).astype(bf16).T

        def clear(_):
            acc[...] = jnp.zeros(acc.shape, f32)

        def start_wo(i):
            start_weights(j + i, woa_hbm, wob_hbm, wo_buf, _S_WO)
            _when(j == _XB_START, lambda: xb_copy().start())

        def wait_wq(i):
            wait_slot(wq_buf, _S_WQ, j + i)
            if i == 1:
                _when(j == _XB_WAIT, lambda: xb_copy().wait())

        ops = {
            "Q": q_proj, "S": qk, "X": softmax, "P": pv, "O": o_proj,
            "Z": clear, "L": stage_lo, "H": stage_hi,
            "k": lambda i: start_pair(_PAIRS_PER_STEP * j + i, ka_hbm, kb_hbm, k_ring, _S_K),
            "v": lambda i: start_pair(_PAIRS_PER_STEP * j + i, va_hbm, vb_hbm, v_ring, _S_V),
            "w": lambda i: start_weights(j + i, wqa_hbm, wqb_hbm, wq_buf, _S_WQ),
            "u": start_wo,
            "x": lambda i: _when(j == 0, lambda: xa_copy(i).start()),
            "l": lambda i: lo_copy(i).start(),
            "h": lambda t: hi_copy(t).start(),
            "a": lambda b: wait_kv(k_ring, _S_K, b),
            "c": lambda b: wait_kv(v_ring, _S_V, b),
            "e": wait_wq,
            "f": lambda i: wait_slot(wo_buf, _S_WO, j + i),
            "y": lambda i: _when(j == 0, lambda: xa_copy(i).wait()),
        }
        for op in program.split():
            ops[op[0]](int(op[1:]))

    run(0, _PROLOGUE)
    lax.fori_loop(0, _NSTEP - 1, lambda j, _: run(j, _STEP), None)
    run(_NSTEP - 1, _LAST_STEP)
    for i in range(2):
        lo_copy(i).wait()
    for t in range(_NTILE):
        hi_copy(t).wait()


@jax.jit
def pallas_concat_heads__gqa_block_cached__mha_block_cached__near_ridge_kernel(
    A_x: jax.Array,
    A_k_cache: jax.Array,
    A_v_cache: jax.Array,
    A_wq: jax.Array,
    A_wo: jax.Array,
    B_x: jax.Array,
    B_k_cache: jax.Array,
    B_v_cache: jax.Array,
    B_wq: jax.Array,
    B_wo: jax.Array,
):
    bf16 = jnp.bfloat16
    out = pl.pallas_call(
        _kernel,
        out_shape=jax.ShapeDtypeStruct((_M, 2 * _D), bf16),
        in_specs=[pl.BlockSpec(memory_space=pl.ANY)] * 10,
        out_specs=pl.BlockSpec(memory_space=pl.ANY),
        scratch_shapes=[
            pltpu.VMEM((2, _M, _D), bf16),
            pltpu.VMEM((_NSTEP, _D, _W), bf16),
            pltpu.VMEM((_NSTEP, _D, _W), bf16),
            pltpu.VMEM((_RING, 2, _SK, _DH), bf16),
            pltpu.VMEM((_RING, 2, _SK, _DH), bf16),
            pltpu.VMEM((_NB, _SQ, _W), bf16),
            pltpu.VMEM((_M, _W), bf16),
            pltpu.VMEM((2 * _D, _M), jnp.float32),
            pltpu.VMEM((_M, _LO), bf16),
            pltpu.VMEM((_M, _HI), bf16),
            pltpu.SemaphoreType.DMA((_NSEM,)),
        ],
        compiler_params=pltpu.CompilerParams(
            vmem_limit_bytes=100 * 2**20,
            flags={"XLA_TPU_RESCHEDULE_DMA_DONES": True},
            disable_bounds_checks=True,
            disable_semaphore_checks=True,
        ),
    )(
        A_x.reshape(_M, _D), A_k_cache, A_v_cache, A_wq, A_wo.T,
        B_x.reshape(_M, _D), B_k_cache, B_v_cache, B_wq, B_wo.T,
    )
    return out.reshape(_NB, _SQ, 2 * _D)
```
